```python
import os as _os
_os.environ.setdefault("JAX_PLATFORMS", "cpu")
import jax
import jax.numpy as jnp

def _softmax(x, axis=-1):
    return jax.nn.softmax(x, axis=axis)
def _gelu(x):
    return jax.nn.gelu(x, approximate=True)
def _silu(x):
    return jax.nn.silu(x)
def _sigmoid(x):
    return jax.nn.sigmoid(x)
def _layernorm(x, axis=-1, eps=1e-5):
    m = jnp.mean(x, axis=axis, keepdims=True)
    v = jnp.var(x, axis=axis, keepdims=True)
    return (x - m) / jnp.sqrt(v + eps)
def _scatter_add(tgt, idx, src, axis=0):
    return tgt.at[idx].add(src)
def _segment_sum(src, seg, n):
    return jax.ops.segment_sum(src, seg, n)
class _Rng:
    def __init__(self, key):
        self._k = key
    def _next(self):
        self._k, sub = jax.random.split(self._k)
        return sub
    def normal(self, shape):
        return jax.random.normal(self._next(), shape, dtype=jnp.bfloat16)
    def randint(self, lo, hi, shape):
        return jax.random.randint(self._next(), shape, lo, hi, dtype=jnp.int32)
    def uniform(self, shape, lo=0.0, hi=1.0):
        return jax.random.uniform(self._next(), shape, jnp.bfloat16, lo, hi)
    def permutation(self, n):
        return jax.random.permutation(self._next(), n)


kernel_name = 'gated_mix__grouped_kv_mqa__glu_gated_reglu__prompt'

def setup_inputs():
    _rng = _Rng(jax.random.key(int.from_bytes(__import__("os").urandom(4), "little")))
    _w = (lambda a: (lambda t: t.astype(jnp.bfloat16) if jnp.issubdtype(t.dtype, jnp.floating) else t)(jnp.asarray(a)))
    def _A_setup():
        B, S, D, H = 1, 2048, 1024, 32
        Dh = D // H
        return {
            "x": _w((lambda *s: _rng.normal(s) * 0.05)(B, S, D)),
            "wq": _w((lambda *s: _rng.normal(s) * 0.2)(D, H * Dh)),
            "wk": _w((lambda *s: _rng.normal(s) * 0.2)(D, Dh)),
            "wv": _w((lambda *s: _rng.normal(s) * 0.05)(D, Dh)),
            "wo": _w((lambda *s: _rng.normal(s) * 0.05)(H * Dh, D)),
        }
    _A_in = _A_setup()

    def _B_setup():
        B, S, D, F = 1, 2048, 1024, 3584
        return {
            "x": _w((lambda *s: _rng.normal(s) * 0.05)(B, S, D)),
            "W_gate": _w((lambda *s: _rng.normal(s) * 0.8)(D, F) * (2.0 / D) ** 0.5),
            "W_up": _w((lambda *s: _rng.normal(s) * 0.8)(D, F) * (2.0 / D) ** 0.5),
            "W_down": _w((lambda *s: _rng.normal(s) * 0.8)(F, D) * (1.0 / F) ** 0.5),
        }
    _B_in = _B_setup()

    return {
        "A_x": _A_in["x"],
        "A_wq": _A_in["wq"],
        "A_wk": _A_in["wk"],
        "A_wv": _A_in["wv"],
        "A_wo": _A_in["wo"],
        "B_x": _B_in["x"],
        "B_W_gate": _B_in["W_gate"],
        "B_W_up": _B_in["W_up"],
        "B_W_down": _B_in["W_down"],
        "gate_w": _w((lambda *s: _rng.normal(s) * 0.05)(1024) * 16.0),
    }

def reference(A_x, A_wq, A_wk, A_wv, A_wo, B_x, B_W_gate, B_W_up, B_W_down, gate_w):
    def _A_ref(x, wq, wk, wv, wo):
        B, S, D = x.shape
        H = 32
        Dh = D // H
        q = (lambda x, *d: x.transpose(*d))((x @ wq).reshape(B, S, H, Dh), 0, 2, 1, 3)
        k = x @ wk
        v = x @ wv
        scores = jnp.einsum("bhqd,bkd->bhqk", q, k) * (Dh ** -0.5)
        p = _softmax(scores, axis=-1)
        o = jnp.einsum("bhqk,bkd->bhqd", p, v)
        return (lambda x, *d: x.transpose(*d))(o, 0, 2, 1, 3).reshape(B, S, H * Dh) @ wo

    def _B_ref(x, W_gate, W_up, W_down):
        gate = jnp.einsum("bsd,df->bsf", x, W_gate)
        up = jnp.einsum("bsd,df->bsf", x, W_up)
        gate = gate * (lambda x, dt: x.astype(dt))(gate > 0, gate.dtype)
        h = gate * up
        return jnp.einsum("bsf,fd->bsd", h, W_down)

    x = A_x
    g = _sigmoid((x * gate_w).sum(-1, keepdims=True))
    a = _A_ref(x, A_wq, A_wk, A_wv, A_wo)
    b = _B_ref(x, B_W_gate, B_W_up, B_W_down)
    return g * a + (1 - g) * b
```

```python
import functools
import math

import jax
import jax.numpy as jnp
from jax import lax
import jax.experimental.pallas as pl
import jax.experimental.pallas.tpu as pltpu

_H = 32
_BF = jnp.bfloat16
_F32 = jnp.float32


def _dot(a, b):
    return jnp.dot(a, b, preferred_element_type=_F32)


def _dot_nt(a, b):
    return lax.dot_general(a, b, (((1,), (1,)), ((), ())), preferred_element_type=_F32)


def _kernel(x_hbm, wq_hbm, wkt_hbm, wvt_hbm, wo_hbm, wg_hbm, wu_hbm, wd_hbm, gw_hbm,
            out_hbm,
            x_v, wq_v, wkv_v, gw_v, wo_v, wg_v, wu_v, wd_v,
            k_v, vt_v, qt_v, ot_v, grow_v, gcol_v,
            s_v, p_v, m_v, l_v, h_v, ob_v, sems, osems, *, S, D, F, TC, FC):
    Dh = D // _H
    NC = S // TC

    x_cp = [pltpu.make_async_copy(x_hbm.at[pl.ds(t * TC, TC)], x_v.at[t], sems.at[t]) for t in range(NC)]
    wk_cp = pltpu.make_async_copy(wkt_hbm, wkv_v.at[pl.ds(0, Dh)], sems.at[NC + 0])
    wv_cp = pltpu.make_async_copy(wvt_hbm, wkv_v.at[pl.ds(Dh, Dh)], sems.at[NC + 1])
    gw_cp = pltpu.make_async_copy(gw_hbm, gw_v, sems.at[NC + 2])
    wq_cp = pltpu.make_async_copy(wq_hbm, wq_v, sems.at[NC + 3])
    wo_cp = pltpu.make_async_copy(wo_hbm, wo_v, sems.at[NC + 4])
    wg_cp = pltpu.make_async_copy(wg_hbm, wg_v, sems.at[NC + 5])
    wu_cp = pltpu.make_async_copy(wu_hbm, wu_v, sems.at[NC + 6])
    wd_cp = pltpu.make_async_copy(wd_hbm, wd_v, sems.at[NC + 7])
    x_cp[0].start(); wk_cp.start(); wv_cp.start(); gw_cp.start(); wq_cp.start()
    for t in range(1, NC):
        x_cp[t].start()

    wk_cp.wait(); wv_cp.wait(); gw_cp.wait()
    gw = gw_v[...].astype(_F32)
    gw_row = jnp.concatenate(
        [jnp.broadcast_to(gw[r:r + 1, :], (128 - 2 * Dh, 128)) for r in range(D // 128)], axis=1)
    wkv_v[pl.ds(2 * Dh, 128 - 2 * Dh), :] = gw_row.astype(_BF)

    qscale = (Dh ** -0.5) * math.log2(math.e)
    for t in range(NC):
        x_cp[t].wait()
        xb = x_v[t]
        kvz = _dot_nt(xb, wkv_v[...])
        k_v[pl.ds(t * TC, TC), :] = kvz[:, :Dh].astype(_BF)
        kvz_t = kvz.T
        vt_v[:, pl.ds(t * TC, TC)] = kvz_t[Dh:2 * Dh].astype(_BF)
        g_row = jax.nn.sigmoid(kvz_t[2 * Dh:2 * Dh + 8])
        grow_v[t] = g_row
        gcol_v[t] = jnp.broadcast_to(1.0 - g_row[:1], (128, TC)).T
        if t == 0:
            wq_cp.wait()
        q = _dot(xb, wq_v[...]) * qscale
        qt_v[t] = q.T.astype(_BF)
        if t == 0:
            wo_cp.start(); wg_cp.start(); wu_cp.start(); wd_cp.start()

    def rows(h):
        return pl.ds(pl.multiple_of(h * Dh, Dh), Dh)

    def step(i, do_a, do_b, do_c):
        for t in range(NC):
            if do_c:
                l_prev = jnp.sum(l_v[t], axis=0, keepdims=True)
                o = _dot(vt_v[...], p_v[t])
                ot_v[t, rows(i - 1), :] = o * (grow_v[t, :1, :] / l_prev)
            if do_b:
                m_prev = jnp.max(m_v[t], axis=0, keepdims=True)
                p = jnp.exp2(s_v[t] - m_prev)
                l_v[t] = jnp.sum(p.reshape(S // 8, 8, TC), axis=0)
                p_v[t] = p.astype(_BF)
            if do_a:
                s = _dot(k_v[...], qt_v[t, rows(i + 1), :])
                s_v[t] = s
                m_v[t] = jnp.max(s.reshape(S // 8, 8, TC), axis=0)

    step(-1, True, False, False)
    step(0, True, True, False)
    lax.fori_loop(1, _H - 1, lambda i, _: step(i, True, True, True), None)
    step(_H - 1, False, True, True)
    step(_H, False, False, True)

    wo_cp.wait(); wg_cp.wait(); wu_cp.wait(); wd_cp.wait()

    def out_cp(t, slot):
        return pltpu.make_async_copy(ob_v.at[slot], out_hbm.at[pl.ds(t * TC, TC)], osems.at[slot])

    def ffn(t, _):
        xb = x_v[t]
        gc = gcol_v[t]
        gc = jnp.concatenate([gc] * (FC // 128), axis=1)
        for f in range(F // FC):
            cs = pl.ds(f * FC, FC)
            gate = _dot(xb, wg_v[:, cs])
            up = _dot(xb, wu_v[:, cs])
            h_v[:, cs] = (jnp.maximum(gate, 0.0) * up * gc).astype(_BF)
        ob = ot_v[t].T.astype(_BF)
        acc = _dot(ob, wo_v[...]) + _dot(h_v[...], wd_v[...])
        ob_v[t] = acc.astype(_BF)
        out_cp(t, t).start()

    lax.fori_loop(0, NC, ffn, None)
    for t in range(NC):
        out_cp(t, t).wait()


@jax.jit
def pallas_gated_mix__grouped_kv_mqa__glu_gated_reglu__prompt_kernel(A_x, A_wq, A_wk, A_wv, A_wo, B_x, B_W_gate, B_W_up, B_W_down, gate_w):
    del B_x
    B, S, D = A_x.shape
    F = B_W_gate.shape[1]
    Dh = D // _H
    TC = 512
    NC = S // TC
    vm = pltpu.VMEM
    out = pl.pallas_call(
        functools.partial(_kernel, S=S, D=D, F=F, TC=TC, FC=512),
        out_shape=jax.ShapeDtypeStruct((S, D), _BF),
        in_specs=[pl.BlockSpec(memory_space=pl.ANY)] * 9,
        out_specs=pl.BlockSpec(memory_space=pl.ANY),
        scratch_shapes=[
            vm((NC, TC, D), _BF), vm((D, D), _BF), vm((128, D), _BF), vm((D // 128, 128), _BF),
            vm((D, D), _BF), vm((D, F), _BF), vm((D, F), _BF), vm((F, D), _BF),
            vm((S, Dh), _BF), vm((Dh, S), _BF), vm((NC, D, TC), _BF), vm((NC, D, TC), _F32),
            vm((NC, 8, TC), _F32), vm((NC, TC, 128), _F32),
            vm((NC, S, TC), _F32), vm((NC, S, TC), _BF), vm((NC, 8, TC), _F32), vm((NC, 8, TC), _F32),
            vm((TC, F), _BF), vm((NC, TC, D), _BF),
            pltpu.SemaphoreType.DMA((NC + 8,)), pltpu.SemaphoreType.DMA((NC,)),
        ],
        compiler_params=pltpu.CompilerParams(vmem_limit_bytes=120 * 2**20),
        name="gated_mix",
    )(A_x.reshape(S, D), A_wq, A_wk.T, A_wv.T, A_wo, B_W_gate, B_W_up, B_W_down,
      gate_w.reshape(D // 128, 128))
    return out.reshape(B, S, D)
```

```python
import functools
import math

import jax
import jax.numpy as jnp
from jax import lax
import jax.experimental.pallas as pl
import jax.experimental.pallas.tpu as pltpu

_H = 32
_BF = jnp.bfloat16
_F32 = jnp.float32
_I32 = jnp.int32
_NZ = 16

_SA = (((1, 1, 0), (1, 1, 1)), ((1, 1, 1),), ((1, 0, 0), (1, 1, 1)), ((1, 0, 0),),
       ((1, 1, 0), (-1, 0, 0)), ((1, 0, 0), (1, 0, 1)), ((1, 0, 1), (-1, 1, 1)))
_SB = (((1, 0, 0),), ((1, 1, 0), (-1, 0, 0)), ((1, 0, 0), (1, 1, 1)), ((1, 0, 1), (-1, 1, 1)),
       ((1, 0, 0), (1, 0, 1)), ((1, 1, 1),), ((1, 1, 0), (1, 1, 1)))
_SC = {(1, 0): ((1, 1), (1, 0)), (1, 1): ((1, 4), (1, 2), (1, 3), (-1, 0)),
       (0, 1): ((1, 5), (1, 3)), (0, 0): ((1, 6), (1, 2), (1, 1), (-1, 5))}


def _dot(a, b):
    return jnp.dot(a, b, preferred_element_type=_F32)


def _dot_nt(a, b):
    return lax.dot_general(a, b, (((1,), (1,)), ((), ())), preferred_element_type=_F32)


def _signed_sum(terms):
    acc = None
    for sign, val in terms:
        if acc is None:
            assert sign > 0
            acc = val
        else:
            acc = acc + val if sign > 0 else acc - val
    return acc


def _factor(terms, load):
    return _signed_sum([(s, load(i, j)) for s, i, j in terms])


def _outer(terms, load):
    return functools.cache(
        lambda i2, j2: _signed_sum([(s, load(2 * i + i2, 2 * j + j2)) for s, i, j in terms]))


def _inner_level(lhs, rhs_outer, emit, before=lambda r2: None):
    prod = []
    for r2 in range(7):
        before(r2)
        a, b = lhs(r2), _factor(_SB[r2], rhs_outer)
        acc = None
        for lo in range(0, b.shape[0], 256):
            part = _dot(a[:, lo:lo + 256].astype(_BF), b[lo:lo + 256].astype(_BF))
            acc = part if acc is None else acc + part
        prod.append(acc)
        for (i2, j2), terms in _SC.items():
            if terms[0][1] == r2:
                emit(i2, j2, _signed_sum([(s, prod[q]) for s, q in terms]))


def _pick(idx, vals):
    acc = vals[-1]
    for r in range(len(vals) - 2, -1, -1):
        acc = jnp.where(idx == r, vals[r], acc)
    return acc


def _after(never, src, dst):
    return pltpu.bitcast(jnp.where(never, pltpu.bitcast(src, _I32), pltpu.bitcast(dst, _I32)), _BF)


def _kernel(x_hbm, wq_hbm, wkt_hbm, wvt_hbm, wo_hbm, wg_hbm, wu_hbm, wd_hbm, gw_hbm,
            out_hbm,
            wd_v, wo_v, m_v, hs_v, k_v, kb_v, vt_v, qt_v, qf_v, grow_v, pe_v, le_v, zero_s,
            sems, wsems, osems, *, S, D, F, NA, NE, cfg):
    Dh = D // _H
    TC = S // 4
    KB = D // 4
    FC = 2 * KB
    NF = F // FC
    NT = F // 4 // 128
    NU = 4 * _H
    SM = S - NA - NE
    vm = pltpu.VMEM

    w2_cp = []
    for j in range(2):
        cols = pl.ds(j * FC, FC)
        w2_cp.append(pltpu.make_async_copy(wd_hbm.at[:, :, cols], wd_v.at[j], sems.at[11 + j]))
        w2_cp.append(pltpu.make_async_copy(wo_hbm.at[:, :, cols], wo_v.at[j], sems.at[13 + j]))

    def rows(h):
        return pl.ds(pl.multiple_of(h * Dh, Dh), Dh)

    def zeros():
        return [zero_s[u] for u in range(_NZ)]

    def vpu_probs(q, slot, lo, n, zs, store):
        for w in range(TC // 128):
            qf_v[slot][0, w] = q[:, w * 128:(w + 1) * 128].astype(_F32)
        steps, sums = [], [None, None]
        for b in range(n // 16):
            for w in range(2):
                acc = None
                for d in range(Dh):
                    kb = kb_v[int(lo == 0)][d + zs[slot % _NZ], pl.ds(16 * b, 16), :]
                    row = jnp.concatenate([qf_v[slot][zs[(2 * b + w) % _NZ], 2 * w + c, pl.ds(d, 8, stride=0), :]
                                           for c in range(2)], axis=1)
                    term = jnp.concatenate([kb, kb], axis=1) * jnp.concatenate([row, row], axis=0)
                    acc = term if acc is None else acc + term
                    steps.append(acc)
                p = jnp.exp2(acc)
                store(pl.ds(16 * b, 16), pl.ds(256 * w, 256), p.astype(_BF))
                part = p[:8] + p[8:]
                sums[w] = part if b == 0 else sums[w] + part
        return jnp.concatenate(sums, axis=1), steps

    def spread_keys(lo, n, zero):
        k = k_v[pl.ds(pl.multiple_of(SM + lo + zero, 16), n), :].astype(_F32)
        done = []
        for d in range(Dh):
            kb = jnp.broadcast_to(k[:, d:d + 1], (n, 128))
            kb_v[int(lo is not NA)][d, pl.ds(lo if lo is not NA else 0, n), :] = kb
            done += [kb[r:r + 8] for r in range(0, n, 8)]
        return done

    def step_at(steps, frac, j):
        acc = steps[max(0, min(len(steps), math.ceil(frac * len(steps))) - 1)]
        r, c = j // 2 * 8 % acc.shape[0], j * 128 % acc.shape[1]
        return acc[r:r + 8, c:c + 128]

    def projections(x_v, xa_v, wb_v, gcol_v, wq_v, wkv_v, gw_v):
        x_cp = [pltpu.make_async_copy(x_hbm.at[pl.ds(t * TC, TC)], x_v.at[t], sems.at[t]) for t in range(4)]
        wq_cp = [[pltpu.make_async_copy(wq_hbm.at[pl.ds(k * FC, FC), pl.ds(j * FC, FC)], wq_v.at[k, j],
                                        sems.at[4 + 2 * k + j]) for j in range(2)] for k in range(2)]
        small_cp = [pltpu.make_async_copy(wkt_hbm, wkv_v.at[pl.ds(0, Dh)], sems.at[8]),
                    pltpu.make_async_copy(wvt_hbm, wkv_v.at[pl.ds(Dh, Dh)], sems.at[9]),
                    pltpu.make_async_copy(gw_hbm, gw_v, sems.at[10])]

        def wb_cp(c, j):
            src = (wg_hbm, wu_hbm)[j]
            return pltpu.make_async_copy(src.at[:, pl.ds(pl.multiple_of(c * FC, FC), FC)],
                                         wb_v.at[c % 2, j], wsems.at[c % 2, j])

        for cp in (*small_cp, x_cp[3], wq_cp[0][0], x_cp[2], wq_cp[1][0], x_cp[1], x_cp[0],
                   wq_cp[1][1], wq_cp[0][1]):
            cp.start()
        for z in range(_NZ):
            zero_s[z] = 0
        qscale = (Dh ** -0.5) * math.log2(math.e)

        def kv_gate(t):
            x, pace = x_v[t], []
            if t == 1 and NE:
                pace = spread_keys(NA, NE, zero_s[0])
            if t == 0 and cfg.get("defer"):
                for blk in range(4):
                    q = m_v[blk][1 + zero_s[0]] + m_v[blk][zero_s[0]]
                    qt_v[2 + blk // 2, pl.ds(blk % 2 * KB, KB), :] = q.T.astype(_BF)
                    pace += [q[lo:lo + 8, 128:] for lo in range(8, TC, 32)]
            if pace:
                cells = [[x[lo:lo + 16, c:c + 128] for c in range(0, D, 128)] for lo in range(0, TC, 16)]
                for g in range(64):
                    c = 4 * (g // 32)
                    cells[g % 32][c] = _after(zero_s[0] > 0, pace[(g + 1) * len(pace) // 64 - 1], cells[g % 32][c])
                x = jnp.concatenate([jnp.concatenate(cc, axis=1) for cc in cells], axis=0)
            kvz = _dot_nt(x, wkv_v[...])
            k = kvz * qscale
            k_v[pl.ds(t * TC, TC), :] = k.astype(_BF)
            kvz_t = kvz.T
            vt_v[t] = kvz_t[Dh:2 * Dh].astype(_BF)
            g_row = jax.nn.sigmoid(kvz_t[2 * Dh:2 * Dh + 8])
            grow_v[t] = g_row
            gcol_v[t] = jnp.broadcast_to(1.0 - g_row[:1], (128, TC)).T

        with jax.named_scope("start"):
            for cp in small_cp:
                cp.wait()
            gw = gw_v[...].astype(_F32)
            gw_row = jnp.concatenate(
                [jnp.broadcast_to(gw[r:r + 1, :], (128 - 2 * Dh, 128)) for r in range(D // 128)], axis=1)
            wkv_v[pl.ds(2 * Dh, 128 - 2 * Dh), :] = gw_row.astype(_BF)
            x_cp[3].wait()

        zero = zero_s[0]
        waits = cfg.get("waits", {0: "q00", 2: "x2", 7: "q10", 14: "x1 x0 q11 q01"})
        kvs = cfg.get("kvs", {0: (3,), 6: (2,), 21: (1, 0)})
        names = {"x0": x_cp[0], "x1": x_cp[1], "x2": x_cp[2], "q00": wq_cp[0][0], "q01": wq_cp[0][1],
                 "q10": wq_cp[1][0], "q11": wq_cp[1][1]}
        with jax.named_scope("proj"):
            for r1 in range(7):
                a_outer = _outer(_SA[r1], lambda i, k: x_v[i + zero, :, pl.ds(k * KB, KB)].astype(_F32))
                b_outer = _outer(_SB[r1], lambda k, j: wq_v[k // 2 + zero, j // 2, pl.ds((k % 2) * KB, KB),
                                                            pl.ds((j % 2) * KB, KB)].astype(_F32))

                def before(r2):
                    for t in kvs.get(7 * r1 + r2, ()):
                        kv_gate(t)
                    for n in waits.get(7 * r1 + r2, "").split():
                        names[n].wait()
                    if 7 * r1 + r2 == cfg.get("wbat", 14):
                        wb_cp(0, 0).start()
                        wb_cp(0, 1).start()

                def lhs(r2):
                    a = _factor(_SA[r2], a_outer)
                    for lo in (0, TC // 2):
                        xa_v[r1][r2, pl.ds(lo, TC // 2), :] = a[lo:lo + TC // 2].astype(_BF)
                    return a

                def emit(i2, j2, cur):
                    if r1 not in (4, 6):
                        m_v[2 * i2 + j2][r1] = cur
                    for (i1, j1), terms in _SC.items():
                        if terms[0][1] == r1 > cfg.get('defer', 0):
                            q = _signed_sum([(s, cur if r == r1 else m_v[2 * i2 + j2][r + zero]) for s, r in terms])
                            qt_v[2 * i1 + i2, pl.ds((2 * j1 + j2) * KB, KB), :] = q.T.astype(_BF)

                _inner_level(lhs, b_outer, emit, before)

        def busy(r1, r2):
            v = 224 + 64 * (len(_SB[r2]) - 1) + {1: 128, 4: 384, 5: 128, 6: 384}.get(r2, 0)
            v += 64 * (2 * len(_SB[r1]) - 1) if r2 < 4 else 0
            return v + (896 if r1 in (4, 6) and r2 in (1, 4, 5, 6) else 0)

        room = [0] + [max(0, cfg.get("cap", 1500) - busy(r // 7, r % 7)) for r in range(1, 49)]
        for cp in w2_cp:
            cp.start()

        with jax.named_scope("ffn1"):
            @pl.loop(0, NF)
            def _(c):
                wb_cp(c, 0).wait()
                wb_cp(c, 1).wait()
                nxt = jnp.minimum(c + 1, NF - 1)

                @pl.when(c + 1 < NF)
                def _():
                    wb_cp(nxt, 0).start()
                    wb_cp(nxt, 1).start()

                zs = zeros()
                zero, never = zs[0], zs[0] > 0
                steps = []
                per = pl.cdiv(NU, NF)
                for u in range(per if NE else 0):
                    unit = jnp.minimum(c * per + u, NU - 1)

                    def store(r, cols, p):
                        pe_v[unit, r, cols] = p

                    le_v[unit], st = vpu_probs(qt_v[unit % 4, rows(unit // 4), :], u, NA, NE, zs, store)
                    steps += st
                nk = pl.cdiv(NA, 16 * NF) * 16
                steps += spread_keys(pl.multiple_of(jnp.minimum(c * nk, NA - nk), 16), nk, zero)

                slot = c % 2
                for r1 in range(7):
                    b_outer = _outer(_SB[r1], lambda k, j: wb_v[slot, j // 2, pl.ds(k * KB, KB), pl.ds((j % 2) * KB, KB)].astype(_F32))

                    def lhs(r2):
                        a = xa_v[r1][r2]
                        r = 7 * r1 + r2
                        if not steps or not room[r]:
                            return a
                        cells = [[a[lo:lo + 16, :128], a[lo:lo + 16, 128:]] for lo in range(0, TC, 16)]
                        n = cfg.get("nt1", 32)
                        for j in range(n):
                            g = (j + 1) * 64 // n - 1
                            src = step_at(steps, (sum(room[:r]) + room[r] * (j + 1) / n) / sum(room), j)
                            cells[g // 2][g % 2] = _after(never, src, cells[g // 2][g % 2])
                        return jnp.concatenate([jnp.concatenate(cc, axis=1) for cc in cells], axis=0)

                    def emit(i2, j2, cur):
                        if r1 not in (4, 6):
                            m_v[2 * i2 + j2][r1] = cur
                        for i1 in range(2):
                            if max(_SC[i1, 0][0][1], _SC[i1, 1][0][1]) == r1:
                                gate, up = (_signed_sum([(s, cur if r == r1 else m_v[2 * i2 + j2][r + zero]) for s, r in _SC[i1, j1]])
                                            for j1 in range(2))
                                i = 2 * i1 + i2
                                hv = jnp.maximum(gate, 0.0) * up
                                for u in range(2):
                                    hs_v[i, 4 * c + 2 * j2 + u] = hv[:, u * 128:(u + 1) * 128] * gcol_v[i]

                    _inner_level(lhs, b_outer, emit)

    pl.run_scoped(
        projections,
        vm((4, TC, D), _BF), [vm((7, TC, KB), _BF)] * 7, vm((2, 2, D, FC), _BF), vm((4, TC, 128), _F32),
        vm((2, 2, FC, FC), _BF), vm((128, D), _BF), vm((D // 128, 128), _BF))

    G = cfg.get("G", 8)

    def attention(ot_v, p_v, l_v, range_v):
        def probs(i, u, zs):
            h, t = i * (G // 4) + u // 4, u % 4
            q = qt_v[t, rows(h), :]
            stores = []
            la, steps = vpu_probs(q, u, 0, NA, zs, lambda *a: stores.append(a))
            kk = [k_v[pl.ds(lo, 16), :] for lo in range(0, SM, 16)]
            g0, g1 = cfg.get("g0", 1), len(kk) - cfg.get("g1", 2)
            for g in range(g0, g1):
                kk[g] = _after(zs[0] > 0, step_at(steps, (g - g0 + 1) / (g1 - g0), g), kk[g])
            p = jnp.exp2(_dot(jnp.concatenate(kk, axis=0)[:, :Dh], q))
            p_v[u][0, pl.ds(0, SM), :] = p.astype(_BF)
            for r, cols, val in stores:
                p_v[u][0, pl.ds(SM + r.start, r.size), cols] = val
            l_v[u][0] = jnp.sum(p.reshape(SM // 8, 8, TC), axis=0) + la

        def values(i, u, zs):
            h, t = i * (G // 4) + u // 4, u % 4
            l, p = l_v[u][zs[0]], p_v[u][zs[0]]
            if NE:
                l, p = l + le_v[4 * h + t], jnp.concatenate([p, pe_v[4 * h + t]], axis=0)
            l = jnp.sum(l, axis=0, keepdims=True)
            o = _dot(jnp.concatenate([vt_v[w] for w in range(4)], axis=1), p)
            ot_v[t, rows(h), :] = o * (grow_v[t, :1, :] / l)
            return l

        def track(ls):
            range_v[0] = functools.reduce(jnp.minimum, ls, range_v[0])
            range_v[1] = functools.reduce(jnp.maximum, ls, range_v[1])

        range_v[...] = jnp.ones_like(range_v)
        with jax.named_scope("attn_pro"):
            @pl.when(zero_s[1] == 0)
            def _():
                zs = zeros()
                for u in range(G):
                    probs(0, u, zs)

        with jax.named_scope("attn_loop"):
            @pl.loop(1, NU // G)
            def _(i):
                zs = zeros()
                ls = []
                for u in range(G):
                    ls.append(values(i - 1, u, zs))
                    probs(i, u, zs)
                track(ls)

        with jax.named_scope("attn_epi"):
            zs = zeros()
            track([values(NU // G - 1, u, zs) for u in range(G)])

        v_max = functools.reduce(jnp.maximum, [jnp.max(jnp.abs(vt_v[w].astype(_F32))) for w in range(4)])
        safe = ((jnp.min(range_v[0]) >= 2.0 ** -40) & (jnp.max(range_v[1]) <= 2.0 ** 40)
                & (v_max <= 2.0 ** 80) & ((v_max >= 2.0 ** -50) | (v_max == 0.0)))
        if cfg.get("force"):
            safe = safe & (zero_s[0] > 0)

        @pl.when(jnp.logical_not(safe))
        def _():
            @pl.loop(0, NU)
            def _(unit):
                h, t = unit // 4, unit % 4
                s = _dot(k_v[:, :Dh], qt_v[t, rows(h), :])
                p = jnp.exp2(s - jnp.max(s, axis=0, keepdims=True))
                o = _dot(jnp.concatenate([vt_v[w] for w in range(4)], axis=1), p.astype(_BF))
                ot_v[t, rows(h), :] = o * (grow_v[t, :1, :] / jnp.sum(p, axis=0, keepdims=True))

    def output(ot_v, ob_v):
        pl.run_scoped(functools.partial(attention, ot_v),
                      [vm((1, SM + NA, TC), _BF)] * G, [vm((1, 8, TC), _F32)] * G, vm((2, 1, TC), _F32))

        for cp in w2_cp:
            cp.wait()

        def dyn_outer(table, r1, load):
            pairs = [t if len(t) == 2 else t * 2 for t in table]
            ia, ja, ib, jb = (_pick(r1, [t[u][v] for t in pairs]) for u in range(2) for v in (1, 2))
            cb = _pick(r1, [float(t[1][0]) if len(t) == 2 else 0.0 for t in table])
            return functools.cache(lambda i2, j2: load(2 * ia + i2, ja, j2) + cb * load(2 * ib + i2, jb, j2))

        def out_cp(slot, i1, j1, i2, j2):
            return pltpu.make_async_copy(
                ob_v.at[slot, i2, j2],
                out_hbm.at[pl.ds(pl.multiple_of((2 * i1 + i2) * TC, TC), TC),
                           pl.ds(pl.multiple_of((2 * j1 + j2) * KB, KB), KB)], osems.at[i2, j2])

        plan = [None] * 7
        for (i1, j1), terms in _SC.items():
            rest = [r for _, r in terms[1:]]
            plan[terms[0][1]] = (i1, j1, *(rest * 3 if len(rest) == 1 else rest))
        for r in range(6, -1, -1):
            plan[r] = plan[r] or (*plan[r + 1][:2], 0, 0, 0)

        with jax.named_scope("ffn2"):
            @pl.loop(0, 7)
            def _(r1):
                i1, j1, ma, mb, mc = (_pick(r1, [p[u] for p in plan]) for u in range(5))
                zs = zeros()
                b_outer = dyn_outer(_SB, r1, lambda k, j, j2: jnp.concatenate(
                    [w[j, k, :, pl.ds(j2 * KB, KB)].astype(_F32) for w in (wd_v, wo_v)], axis=0))

                def lhs(r2):
                    z = zs[r2]
                    h_outer = dyn_outer(_SA, r1, lambda i, k, k2: jnp.concatenate(
                        [hs_v[i + z, (2 * k + k2) * NT + u] for u in range(NT)], axis=1))
                    o_outer = dyn_outer(_SA, r1, lambda i, k, k2: ot_v[
                        i + z, pl.ds(pl.multiple_of((2 * k + k2) * KB, KB), KB), :])
                    return jnp.concatenate([_factor(_SA[r2], h_outer), _factor(_SA[r2], o_outer).T], axis=1)

                def emit(i2, j2, cur):
                    m = m_v[2 * i2 + j2]
                    step = cfg.get("piece", 32)
                    for lo in range(0, TC, step):
                        rs = pl.ds(lo, step)
                        val = (cur[lo:lo + step] + m[ma, rs]) + (m[mb, rs] - m[mc, rs])
                        ob_v[r1 % 2, i2, j2, rs, :] = val.astype(_BF)
                        m[r1, rs] = cur[lo:lo + step]

                _inner_level(lhs, b_outer, emit)

                @pl.when(r1 > 0)
                def _():
                    for i2 in range(2):
                        for j2 in range(2):
                            out_cp(r1 % 2, i1, j1, i2, j2).wait()

                for i2 in range(2):
                    for j2 in range(2):
                        out_cp(r1 % 2, i1, j1, i2, j2).start()

        with jax.named_scope("outwait"):
            for i2 in range(2):
                for j2 in range(2):
                    out_cp(0, 0, 0, i2, j2).wait()

    pl.run_scoped(output, vm((4, D, TC), _F32), vm((2, 2, 2, TC, KB), _BF))


def make(NA=128, NE=80, **cfg):
    @jax.jit
    def kernel(A_x, A_wq, A_wk, A_wv, A_wo, B_x, B_W_gate, B_W_up, B_W_down, gate_w):
        del B_x
        B, S, D = A_x.shape
        F = B_W_gate.shape[1]
        Dh = D // _H
        TC, KB = S // 4, D // 4
        FC = 2 * KB
        vm = pltpu.VMEM
        out = pl.pallas_call(
            functools.partial(_kernel, S=S, D=D, F=F, NA=NA, NE=NE, cfg=cfg),
            out_shape=jax.ShapeDtypeStruct((S, D), _BF),
            in_specs=[pl.BlockSpec(memory_space=pl.ANY)] * 9,
            out_specs=pl.BlockSpec(memory_space=pl.ANY),
            scratch_shapes=[
                vm((2, 4, F // 4, FC), _BF), vm((2, 4, KB, FC), _BF), [vm((7, TC, KB), _F32)] * 4,
                vm((4, F // 128, TC, 128), _F32),
                vm((S, 128), _BF), [vm((Dh, max(NE, 16), 128), _F32), vm((Dh, NA, 128), _F32)], vm((4, Dh, TC), _BF), vm((4, D, TC), _BF),
                [vm((1, TC // 128, Dh, 128), _F32)] * pl.cdiv(4 * _H, F // FC), vm((4, 8, TC), _F32),
                vm((4 * _H, max(NE, 16), TC), _BF), vm((4 * _H, 8, TC), _F32),
                pltpu.SMEM((_NZ,), jnp.int32),
                pltpu.SemaphoreType.DMA((15,)), pltpu.SemaphoreType.DMA((2, 2)), pltpu.SemaphoreType.DMA((2, 2)),
            ],
            compiler_params=pltpu.CompilerParams(vmem_limit_bytes=127 * 2**20),
            name="gated_mix",
        )(A_x.reshape(S, D), A_wq, A_wk.T, A_wv.T, A_wo.reshape(4, KB, D), B_W_gate, B_W_up,
          B_W_down.reshape(4, F // 4, D), gate_w.reshape(D // 128, 128))
        return out.reshape(B, S, D)
    return kernel


pallas_gated_mix__grouped_kv_mqa__glu_gated_reglu__prompt_kernel = make()
```

```python
import functools
import math

import jax
import jax.numpy as jnp
import numpy as np
from jax import lax
import jax.experimental.pallas as pl
import jax.experimental.pallas.tpu as pltpu

_HEADS = 32
_X_STEPS = 8
_UNITS = 8
_VPU_KEYS = (32, 32, 32, 32, 16)
_ZEROS = 16

_BF = jnp.bfloat16
_F32 = jnp.float32

_SA = (((1, 1, 0), (1, 1, 1)), ((1, 1, 1),), ((1, 0, 0), (1, 1, 1)), ((1, 0, 0),),
       ((1, 1, 0), (-1, 0, 0)), ((1, 0, 0), (1, 0, 1)), ((1, 0, 1), (-1, 1, 1)))
_SB = (((1, 0, 0),), ((1, 1, 0), (-1, 0, 0)), ((1, 0, 0), (1, 1, 1)), ((1, 0, 1), (-1, 1, 1)),
       ((1, 0, 0), (1, 0, 1)), ((1, 1, 1),), ((1, 1, 0), (1, 1, 1)))
_SC = {(1, 0): ((1, 1), (1, 0)), (1, 1): ((1, 4), (1, 2), (1, 3), (-1, 0)),
       (0, 1): ((1, 5), (1, 3)), (0, 0): ((1, 6), (1, 2), (1, 1), (-1, 5))}
_IN_ORDER = (0, 1, 2, 3, 4, 5, 6)
_MIDDLE_ORDER = (5, 3, 0, 1, 2, 4, 6)
_INNER_ORDER = (0, 1, 2, 4, 3, 5, 6)


def _dot(a, b):
    return jnp.dot(a, b, preferred_element_type=_F32)


def _dot_nt(a, b):
    return lax.dot_general(a, b, (((1,), (1,)), ((), ())), preferred_element_type=_F32)


def _signed_sum(terms):
    (sign, acc), *rest = terms
    assert sign > 0
    for sign, val in rest:
        acc = acc + val if sign > 0 else acc - val
    return acc


def _factor(terms, blk):
    return _signed_sum([(s, blk(i, j)) for s, i, j in terms])


def _block_factor(terms, blk, n):
    return functools.cache(lambda i2, j2: _factor(terms, lambda i, j: blk(n * i + i2, n * j + j2)))


def _quadrants(m):
    h, w = m.shape[0] // 2, m.shape[1] // 2
    return lambda i, j: m[i * h:(i + 1) * h, j * w:(j + 1) * w]


def _completed(r, done):
    return [(ij, terms) for ij, terms in _SC.items()
            if r in [q for _, q in terms] and all(q in done for _, q in terms)]


def _when_complete(order, product, emit):
    prod = {}
    for r in order:
        prod[r] = product(r)
        for ij, terms in _completed(r, prod):
            terms = [t for t in terms if t[1] == r] + [t for t in terms if t[1] != r]
            emit(*ij, _signed_sum([(s, prod[q]) for s, q in terms]))


def _accumulate(order, product, emit):
    out, done = {}, []
    for r in order:
        val = product(r)
        done.append(r)
        for ij, terms in _SC.items():
            for sign in (s for s, q in terms if q == r):
                out[ij] = (sign, val) if ij not in out else (
                    1, _signed_sum(sorted([out[ij], (sign, val)], key=lambda t: -t[0])))
        for ij, _ in _completed(r, done):
            emit(*ij, out[ij][1])


def _after(never, steps, frac, j, dst):
    src = steps[min(len(steps), math.ceil(frac * len(steps))) - 1]
    r, c = j // 2 * 8 % src.shape[0], j * 128 % src.shape[1]
    src = pltpu.bitcast(src[r:r + 8, c:c + 128], jnp.int32)
    return pltpu.bitcast(jnp.where(never, src, pltpu.bitcast(dst, jnp.int32)), _BF)


def _kernel(x_hbm, wq_hbm, wkt_hbm, wvt_hbm, wo_hbm, wg_hbm, wu_hbm, wd_hbm, gw_hbm, out_hbm,
            wd_v, wo_v, h_v, k_v, kf_v, vt_v, qt_v, g_v, mo_v, zero_s, sems):
    S, D = out_hbm.shape
    F = wg_hbm.shape[1]
    Dh = D // _HEADS
    TR = S // 4
    TC = D // 4
    FC = 2 * TC
    SM = S - sum(_VPU_KEYS)
    vmem = pltpu.VMEM
    wq_sems, wb_sems = (sems.at[_X_STEPS], sems.at[_X_STEPS + 1]), _X_STEPS + 2
    small_sem, w2_sem, out_sem = (sems.at[_X_STEPS + 4 + i] for i in range(3))

    w2_copies = [pltpu.make_async_copy(src.at[:, :, pl.ds(j * FC, FC)], dst.at[j], w2_sem)
                 for j in range(2) for src, dst in ((wd_hbm, wd_v), (wo_hbm, wo_v))]

    def zeros():
        return [zero_s[u] for u in range(_ZEROS)]

    def spread_keys(b, zero):
        n = _VPU_KEYS[b] // 2
        k = k_v[pl.ds(pl.multiple_of(SM + sum(_VPU_KEYS[:b]) + zero, 16), 2 * n), :].astype(_F32)
        for d in range(Dh // 2):
            wide = [jnp.broadcast_to(k[:, c:c + 1], (2 * n, 128)) for c in (d, Dh // 2 + d)]
            for r in range(7):
                kf_v[b][r * Dh // 2 + d] = _factor(_SA[r], lambda i, c: wide[c][n * i:n * (i + 1)])

    def projections(x_v, xf_v, wb_v, m_v, kvz_v, ng_v, wkv_v, gw_v):
        def x_copy(g):
            return pltpu.make_async_copy(x_hbm.at[:, g], x_v.at[g], sems.at[g])

        def wq_copy(k, j):
            return pltpu.make_async_copy(wq_hbm.at[pl.ds(k * FC, FC), pl.ds(j * FC, FC)],
                                         wb_v.at[1, j, pl.ds(k * FC, FC)], wq_sems[min(1, k + j)])

        def wb_copies(c):
            return [pltpu.make_async_copy(w.at[:, pl.ds(pl.multiple_of(c * FC, FC), FC)],
                                          wb_v.at[c % 2, j], sems.at[wb_sems + c % 2])
                    for j, w in enumerate((wg_hbm, wu_hbm))]

        small_copies = [pltpu.make_async_copy(wkt_hbm, wkv_v.at[pl.ds(0, Dh)], small_sem),
                        pltpu.make_async_copy(wvt_hbm, wkv_v.at[pl.ds(Dh, Dh)], small_sem),
                        pltpu.make_async_copy(gw_hbm, gw_v.at[pl.ds(0, D // 128)], small_sem)]
        wq_rest = [wq_copy(1, 0), wq_copy(1, 1), wq_copy(0, 1)]
        for copy in (*small_copies, *map(x_copy, range(_X_STEPS)), wq_copy(0, 0), *wq_rest):
            copy.start()
        for u in range(_ZEROS):
            zero_s[u] = 0
        for m in mo_v:
            m[0] = jnp.zeros((TR, TC), _F32)
        for copy in small_copies:
            copy.wait()
        gw = gw_v[pl.ds(0, D // 128), :].astype(_F32)
        wkv_v[pl.ds(2 * Dh, 128 - 2 * Dh), :] = jnp.concatenate(
            [jnp.broadcast_to(gw[r:r + 1, :], (128 - 2 * Dh, 128)) for r in range(D // 128)],
            axis=1).astype(_BF)

        RG = S // 8 // _X_STEPS

        @pl.loop(0, _X_STEPS)
        def _(g):
            x_copy(g).wait()
            zs, steps = zeros(), []
            for lo in range(0, RG, 8):
                for r1 in range(7):
                    z = zs[(lo // 8 * 7 + r1) % _ZEROS]
                    pair = functools.cache(
                        lambda i, k: x_v[g + z, i, pl.ds(lo, 8), pl.ds(256 * k, 256)].astype(_F32))
                    a1 = _block_factor(
                        _SA[r1], lambda i, k: pair(i, k // 2)[:, k % 2 * 128:k % 2 * 128 + 128], 4)
                    for r2 in range(7):
                        a2 = _block_factor(_SA[r2], a1, 2)
                        a3 = [_factor(terms, a2) for terms in _SA] + [a2(1, 0)]
                        for u in range(4):
                            xf_v[r1][r2, u, pl.ds(pl.multiple_of(g * RG + lo, 8), 8), :] = (
                                jnp.concatenate(a3[2 * u:2 * u + 2], axis=1).astype(_BF))
                        steps.append(a3[2])
            x = x_v[g].reshape(8 * RG, D)
            tiles = [[x[lo:lo + 16, c:c + 128] for c in range(0, D, 128)]
                     for lo in range(0, 8 * RG, 16)]
            n = 8 * len(tiles)
            for j in range(n):
                r, c = j // 4 % len(tiles), j // (n // 2) * 4 + j % 4
                tiles[r][c] = _after(zs[0] > 0, steps, 0.9 * (j + 1) / n, 0, tiles[r][c])
            x = jnp.concatenate([jnp.concatenate(row, axis=1) for row in tiles], axis=0)
            kvz_v[pl.ds(pl.multiple_of(g * 8 * RG, 8 * RG), 8 * RG), :] = _dot_nt(x, wkv_v[...])

        def seven_products(a, b):
            out = {}
            _accumulate(_INNER_ORDER,
                        lambda r: _dot(a(r), _factor(_SB[r], _quadrants(b)).astype(_BF)),
                        lambda i, j, blk: out.update({(i, j): blk}))
            return jnp.concatenate(
                [jnp.concatenate([out[i, 0], out[i, 1]], axis=1) for i in range(2)], axis=0)

        def eight_products(a, b):
            top = jnp.concatenate([b[:128] - b[128:], b[128:]], axis=0)
            return jnp.concatenate(
                [_dot(jnp.concatenate([a(3), a(5)], axis=1), top.astype(_BF)),
                 _dot(jnp.concatenate([a(7), a(1)], axis=1), b.astype(_BF))], axis=0)

        def project(slot, zs, inner, emit, before=lambda r1: None):
            for r1 in range(7):
                before(r1)

                @functools.cache
                def b1(z):
                    return _block_factor(_SB[r1], lambda k, j: wb_v[
                        slot + zs[z], j // 2, pl.ds(k * TC, TC), pl.ds(j % 2 * TC, TC)].astype(_F32), 2)

                def middle(r2):
                    z = r1 if len(_SB[r1]) > 1 else (7 * r1 + r2) % _ZEROS
                    return inner(lambda r3: xf_v[r1][r2, r3 // 2, :, pl.ds(r3 % 2 * 128, 128)],
                                 _factor(_SB[r2], b1(z)))

                _when_complete(_MIDDLE_ORDER, middle, functools.partial(emit, r1))

        zs = zeros()

        def before(r1):
            if r1 == 0:
                wq_copy(0, 0).wait()
            if r1 == 1:
                for copy in wq_rest:
                    copy.wait()
                for copy in wb_copies(0):
                    copy.start()
            if r1 in (0, 2, 3, 5):
                t = {0: 3, 2: 0, 3: 1, 5: 2}[r1]
                kvz = jnp.concatenate([kvz_v[pl.ds((8 * g + b) * RG, RG), :]
                                       for b in (2 * t, 2 * t + 1) for g in range(_X_STEPS)], axis=0)
                k_v[pl.ds(t * TR, TR), :] = (kvz * (Dh ** -0.5 * math.log2(math.e))).astype(_BF)
                kvz_t = kvz.T
                vt_v[t] = kvz_t[Dh:2 * Dh].astype(_BF)
                g_v[t] = g = jax.nn.sigmoid(kvz_t[2 * Dh:2 * Dh + 8])
                ng_v[t] = jnp.broadcast_to(1.0 - g[:1], (128, TR)).T
            if r1 == 3:
                spread_keys(0, zs[0])

        def emit_q(r1, i2, j2, cur):
            m = m_v[2 * i2 + j2]
            if r1 not in (4, 6):
                m[r1][0] = cur
            for (i1, j1), terms in _SC.items():
                if terms[0][1] == r1:
                    q = _signed_sum([(s, cur if r == r1 else m[r][zs[r1]]) for s, r in terms])
                    qt_v[2 * i1 + i2, pl.ds((2 * j1 + j2) * TC, TC), :] = q.T.astype(_BF)

        project(1, zs, eight_products, emit_q, before)

        @pl.loop(0, F // FC)
        def _(c):
            for copy in wb_copies(c):
                copy.wait()

            @pl.when(c + 1 < F // FC)
            def _():
                for copy in wb_copies(c + 1):
                    copy.start()

            zs = zeros()

            def emit_h(r1, i2, j2, cur):
                m = m_v[2 * i2 + j2]

                def get(r):
                    return m[r][zs[r1]]

                if r1 == 2:
                    m[4][0] = cur - get(0)
                    m[2][0] = cur + get(1)
                elif r1 not in (4, 6):
                    m[r1][0] = cur
                elif r1 == 4:
                    gate, up = get(0) + get(1), (cur + get(4)) + get(3)
                    ng = jnp.concatenate([ng_v[2 + i2]] * 2, axis=1)
                    store_h(2 + i2, j2, up * (jnp.maximum(gate, 0.0) * ng))
                else:
                    gate, up = (cur + get(2)) - get(5), get(5) + get(3)
                    ng = jnp.concatenate([ng_v[i2]] * 2, axis=1)
                    store_h(i2, j2, jnp.maximum(gate, 0.0) * (up * ng))

            def store_h(i, j2, h):
                for u in range(2):
                    h_v[i, 4 * c + 2 * j2 + u] = h[:, u * 128:(u + 1) * 128]

            project(c % 2, zs, seven_products, emit_h)

    pl.run_scoped(
        projections,
        vmem((_X_STEPS, 8, S // 8 // _X_STEPS, D), _BF), [vmem((7, 4, S // 8, 256), _BF)] * 7,
        vmem((2, 2, D, FC), _BF), [[vmem((1, TR, TC), _F32)] * 6] * 4, vmem((S, 128), _F32),
        vmem((4, TR, 128), _F32), vmem((128, D), _BF), vmem((64, 128), _BF))

    def attention(ot_v, align_v, qf_v, p_v, l_v, range_v):
        def head_rows(h):
            return pl.ds(pl.multiple_of(h * Dh, Dh), Dh)

        def vpu_probs(q, u, zs):
            half = Dh // 2
            factors = [_factor(terms, _quadrants(q.astype(_F32))) for terms in _SB]
            steps, sums, blocks = [], {}, []
            for b, kf in enumerate(kf_v):
                n, lo, out = _VPU_KEYS[b] // 16, sum(_VPU_KEYS[:b]), {}

                def product(r):
                    acc = None
                    for d in range(half):
                        col = kf[r * half + d + zs[u]]
                        if b == 0:
                            row = jnp.broadcast_to(factors[r][d:d + 1], (8, TR // 2))
                            qf_v[u][r * half + d] = row
                        else:
                            row = qf_v[u][r * half + d + zs[b]]
                        term = jnp.concatenate([col, col], axis=1) * jnp.concatenate([row] * n, axis=0)
                        acc = term if acc is None else acc + term
                        steps.extend([acc] * (8 * n + 4 * (b == 0) + 8 * (d == 0)))
                    return acc

                def emit(i, j, s):
                    p = out[i, j] = jnp.exp2(s)
                    for part in (p[8 * w:8 * w + 8] for w in range(n)):
                        sums[j] = sums[j] + part if j in sums else part
                    if n == 2:
                        blocks.append((lo + 16 * i, 256 * j, p))
                    elif (1 - i, j) in out:
                        blocks.append((lo, 256 * j, jnp.concatenate([out[0, j], out[1, j]], axis=0)))

                _accumulate(_IN_ORDER, product, emit)
            return jnp.concatenate([sums[0], sums[1]], axis=1), steps, blocks

        def probs(i, u, zs):
            q = qt_v[u % 4, head_rows(i * (_UNITS // 4) + u // 4), :]
            vpu_sum, steps, blocks = vpu_probs(q, u, zs)
            k = [k_v[pl.ds(lo, 16), :] for lo in range(0, SM, 16)]
            for j in range(len(k) - 2):
                k[j] = _after(zs[0] > 0, steps, (j + 1) / (len(k) - 2), j, k[j])
            p = jnp.exp2(_dot(jnp.concatenate(k, axis=0)[:, :Dh], q))
            p_v[u][0, pl.ds(0, SM), :] = p.astype(_BF)
            for r, c, blk in blocks:
                p_v[u][0, pl.ds(SM + r, 16), pl.ds(c, 256)] = blk.astype(_BF)
            l_v[u][0] = jnp.sum(p.reshape(SM // 8, 8, TR), axis=0) + vpu_sum

        def values(h, t, p, l):
            o = _dot(jnp.concatenate([vt_v[w] for w in range(4)], axis=1), p)
            ot_v[t, head_rows(h), :] = o * (g_v[t, :1, :] / l)

        def stored_values(i, u, zs):
            l = jnp.sum(l_v[u][zs[0]], axis=0, keepdims=True)
            values(i * (_UNITS // 4) + u // 4, u % 4, p_v[u][zs[0]], l)
            return l

        def track(sums):
            range_v[0] = functools.reduce(jnp.minimum, sums, range_v[0])
            range_v[1] = functools.reduce(jnp.maximum, sums, range_v[1])

        range_v[...] = jnp.ones_like(range_v)
        align_v[0] = jnp.zeros((8, 128), _F32)

        @pl.when(zero_s[1] == 0)
        def _():
            zs = zeros()
            for b in range(1, len(kf_v)):
                spread_keys(b, zs[0])
            for u in range(_UNITS):
                probs(0, u, zs)

        for copy in w2_copies:
            copy.start()

        @pl.loop(1, 4 * _HEADS // _UNITS)
        def _(i):
            zs, sums = zeros(), []
            for u in range(_UNITS):
                sums.append(stored_values(i - 1, u, zs))
                probs(i, u, zs)
            track(sums)

        zs = zeros()
        track([stored_values(4 * _HEADS // _UNITS - 1, u, zs) for u in range(_UNITS)])

        v_max = jnp.max(jnp.max(jnp.abs(vt_v[...].astype(_F32)), axis=0), keepdims=True)
        v_max = v_max + align_v[zero_s[0], :1, :1]
        safe = ((range_v[0] >= 2.0 ** -40) & (range_v[1] <= 2.0 ** 40)
                & (v_max <= 2.0 ** 80) & ((v_max >= 2.0 ** -50) | (v_max == 0.0)))

        @pl.when(jnp.max(jnp.where(safe, 0.0, 1.0)) > 0.0)
        def _():
            def plain_q(x_v, w_v):
                pltpu.sync_copy(x_hbm, x_v)
                for j in range(4):
                    pltpu.sync_copy(wq_hbm.at[:, pl.ds(j * TC, TC)], w_v.at[j])

                @pl.loop(0, 16)
                def _(n):
                    t, j = n // 4, n % 4
                    q = _dot(x_v[pl.ds(2 * t, 2)].reshape(TR, D), w_v[j])
                    qt_v[t, pl.ds(pl.multiple_of(j * TC, TC), TC), :] = q.T.astype(_BF)

            pl.run_scoped(plain_q, vmem(x_hbm.shape, _BF), vmem((4, D, TC), _BF))

            @pl.loop(0, 4 * _HEADS)
            def _(unit):
                h, t = unit // 4, unit % 4
                s = _dot(k_v[:, :Dh], qt_v[t, head_rows(h), :])
                p = jnp.exp2(s - jnp.max(s, axis=0, keepdims=True))
                values(h, t, p.astype(_BF), jnp.sum(p, axis=0, keepdims=True))

    def output(ot_v, out_v):
        pl.run_scoped(functools.partial(attention, ot_v),
                      vmem((1, 8, 128), _F32),
                      [vmem((7 * Dh // 2, 8, TR // 2), _F32)] * _UNITS,
                      [vmem((1, S, TR), _BF)] * _UNITS, [vmem((1, 8, TR), _F32)] * _UNITS,
                      vmem((2, 8, TR), _F32))
        for copy in w2_copies:
            copy.wait()

        def out_copy(i1, j1, i2, j2):
            return pltpu.make_async_copy(
                out_v[2 * i2 + j2].at[2 * i1 + j1],
                out_hbm.at[pl.ds(pl.multiple_of((2 * i1 + i2) * TR, TR), TR),
                           pl.ds(pl.multiple_of((2 * j1 + j2) * TC, TC), TC)], out_sem)

        def factor_spec(terms):
            (_, ia, ja), (sign, ib, jb) = terms[0], terms[-1]
            return (*map(np.int32, (ia, ja, ib, jb)), np.float32(sign if len(terms) == 2 else 0))

        def outer_factor(spec, blk):
            ia, ja, ib, jb, coef = spec
            return functools.cache(
                lambda i2, j2: blk(2 * ia + i2, ja, j2) + coef * blk(2 * ib + i2, jb, j2))

        plan = [None] * 7
        for (i1, j1), terms in _SC.items():
            rest = [r for _, r in terms[1:]]
            plan[terms[0][1]] = (1, i1, j1, *(rest * 3 if len(rest) == 1 else rest))
        for r in reversed(range(7)):
            plan[r] = plan[r] or (0, *plan[r + 1][1:3], 0, 0, 0)
        specs = [(factor_spec(_SA[r]), factor_spec(_SB[r]), tuple(map(np.int32, plan[r])))
                 for r in range(7)]

        def step(spec, keep=None, before=lambda r2: None):
            spec_a, spec_b, (_, i1, j1, ma, mb, mc) = spec
            zs = zeros()
            b1 = outer_factor(spec_b, lambda k, j, j2: jnp.concatenate(
                [w[j, k, :, pl.ds(j2 * TC, TC)].astype(_F32) for w in (wd_v, wo_v)], axis=0))

            @functools.cache
            def a1(z):
                n = F // 4 // 128
                return (outer_factor(spec_a, lambda i, k, k2: jnp.concatenate(
                            [h_v[i + zs[z], (2 * k + k2) * n + u] for u in range(n)], axis=1)),
                        outer_factor(spec_a, lambda i, k, k2: ot_v[
                            i + zs[z], pl.ds(pl.multiple_of((2 * k + k2) * TC, TC), TC), :]))

            def product(r2):
                before(r2)
                shared = r2 if keep is None else 7
                h, ot = (_factor(_SA[r2], lambda i, k: a1(shared if i == k == 1 else r2)[w](i, k))
                         for w in range(2))
                a, b = jnp.concatenate([h, ot.T], axis=1), _factor(_SB[r2], b1)
                return functools.reduce(jnp.add, (
                    _dot(a[:, lo:lo + 256].astype(_BF), b[lo:lo + 256].astype(_BF))
                    for lo in range(0, b.shape[0], 256)))

            def emit(i2, j2, cur):
                m, n = mo_v[2 * i2 + j2], TR if keep is None else 64
                for lo in range(0, TR, n):
                    rows, part = pl.ds(lo, n), cur[lo:lo + n]
                    val = (part + m[ma, rows]) + (m[mb, rows] - m[mc, rows])
                    out_v[2 * i2 + j2][2 * i1 + j1, rows, :] = val.astype(_BF)
                    if keep is not None:
                        m[keep, rows] = part

            _when_complete(_IN_ORDER, product, emit)

        @pl.loop(0, 6, init_carry=specs[0])
        def _(r1, spec):
            step(spec, keep=r1)
            final, i1, j1 = spec[2][:3]

            @pl.when(final > 0)
            def _():
                for i2, j2 in _SC:
                    out_copy(i1, j1, i2, j2).start()

            return jax.tree.map(
                lambda *v: functools.reduce(
                    lambda acc, r: jnp.where(r1 + 1 == r, v[r], acc), range(1, 5), v[5]),
                *specs)

        def send_finished_blocks(r2):
            if r2 == 6:
                @pl.loop(0, 1 + zero_s[0])
                def _(_):
                    for i2, j2 in list(_SC)[:3]:
                        out_copy(0, 0, i2, j2).start()

        step(specs[6], before=send_finished_blocks)
        out_copy(0, 0, 0, 0).start()
        for i1, j1 in _SC:
            for i2, j2 in _SC:
                out_copy(i1, j1, i2, j2).wait()

    pl.run_scoped(output, vmem((4, D, TR), _F32), [vmem((4, TR, TC), _BF)] * 4)


@jax.jit
def pallas_gated_mix__grouped_kv_mqa__glu_gated_reglu__prompt_kernel(
    A_x: jax.Array,
    A_wq: jax.Array,
    A_wk: jax.Array,
    A_wv: jax.Array,
    A_wo: jax.Array,
    B_x: jax.Array,
    B_W_gate: jax.Array,
    B_W_up: jax.Array,
    B_W_down: jax.Array,
    gate_w: jax.Array,
):
    del B_x
    B, S, D = A_x.shape
    F = B_W_gate.shape[1]
    Dh, TR, TC = D // _HEADS, S // 4, D // 4
    assert (B, S, D) == (1, 2048, 1024) and F % (2 * TC) == 0
    vmem = pltpu.VMEM
    out = pl.pallas_call(
        _kernel,
        out_shape=jax.ShapeDtypeStruct((S, D), _BF),
        in_specs=[pl.BlockSpec(memory_space=pl.ANY)] * 9,
        out_specs=pl.BlockSpec(memory_space=pl.ANY),
        scratch_shapes=[
            vmem((2, 4, F // 4, 2 * TC), _BF),
            vmem((2, 4, TC, 2 * TC), _BF),
            vmem((4, F // 128, TR, 128), _F32),
            vmem((S, 128), _BF),
            [vmem((7 * Dh // 2, n // 2, 128), _F32) for n in _VPU_KEYS],
            vmem((4, Dh, TR), _BF),
            vmem((4, D, TR), _BF),
            vmem((4, 8, TR), _F32),
            [vmem((7, TR, TC), _F32)] * 4,
            pltpu.SMEM((_ZEROS,), jnp.int32),
            pltpu.SemaphoreType.DMA((_X_STEPS + 7,)),
        ],
        compiler_params=pltpu.CompilerParams(vmem_limit_bytes=127 * 2**20),
        name="gated_mix",
    )(A_x.reshape(8, _X_STEPS, S // 8 // _X_STEPS, D), A_wq, A_wk.T, A_wv.T,
      A_wo.reshape(4, TC, D), B_W_gate, B_W_up, B_W_down.reshape(4, F // 4, D),
      gate_w.reshape(D // 128, 128))
    return out.reshape(B, S, D)
```

```python
import functools
import math

import jax
import jax.numpy as jnp
import numpy as np
from jax import lax
import jax.experimental.pallas as pl
import jax.experimental.pallas.tpu as pltpu

_HEADS = 32
_X_STEPS = 8
_UNITS = 8
_VPU_GROUPS = 5
_ZEROS = 16

_BF = jnp.bfloat16
_F32 = jnp.float32

_SA = (((1, 1, 0), (1, 1, 1)), ((1, 1, 1),), ((1, 0, 0), (1, 1, 1)), ((1, 0, 0),),
       ((1, 1, 0), (-1, 0, 0)), ((1, 0, 0), (1, 0, 1)), ((1, 0, 1), (-1, 1, 1)))
_SB = (((1, 0, 0),), ((1, 1, 0), (-1, 0, 0)), ((1, 0, 0), (1, 1, 1)), ((1, 0, 1), (-1, 1, 1)),
       ((1, 0, 0), (1, 0, 1)), ((1, 1, 1),), ((1, 1, 0), (1, 1, 1)))
_SC = {(1, 0): ((1, 1), (1, 0)), (1, 1): ((1, 4), (1, 2), (1, 3), (-1, 0)),
       (0, 1): ((1, 5), (1, 3)), (0, 0): ((1, 6), (1, 2), (1, 1), (-1, 5))}
_IN_ORDER = (0, 1, 2, 3, 4, 5, 6)
_MIDDLE_ORDERS = ((5, 3, 1, 0, 2, 4, 6), (5, 6, 3, 0, 1, 2, 4), (5, 3, 0, 2, 1, 4, 6),
                  (5, 0, 3, 1, 2, 4, 6), (3, 0, 6, 5, 1, 2, 4), (0, 3, 2, 4, 5, 1, 6),
                  (5, 3, 0, 1, 2, 4, 6))
_INNER_ORDERS = ((0, 6, 1, 2, 4, 3, 5), (0, 1, 2, 4, 3, 5, 6), (0, 1, 2, 4, 3, 5, 6),
                 (0, 1, 2, 3, 5, 4, 6))
_OUTPUT_ORDER = (0, 3, 1, 2, 5, 4, 6)
_VPU_ORDERS = ((0, 1, 2, 3, 5, 4, 6), (0, 1, 2, 4, 3, 5, 6), (0, 1, 2, 4, 3, 5, 6),
               (0, 1, 2, 4, 3, 5, 6), (0, 1, 2, 3, 4, 6, 5))


def _dot(a, b):
    return jnp.dot(a, b, preferred_element_type=_F32)


def _dot_nt(a, b):
    return lax.dot_general(a, b, (((1,), (1,)), ((), ())), preferred_element_type=_F32)


def _signed_sum(terms):
    (sign, acc), *rest = terms
    assert sign > 0
    for sign, val in rest:
        acc = acc + val if sign > 0 else acc - val
    return acc


def _factor(terms, blk):
    return _signed_sum([(s, blk(i, j)) for s, i, j in terms])


def _block_factor(terms, blk, n):
    return functools.cache(lambda i2, j2: _factor(terms, lambda i, j: blk(n * i + i2, n * j + j2)))


def _quadrants(m):
    h, w = m.shape[0] // 2, m.shape[1] // 2
    return lambda i, j: m[i * h:(i + 1) * h, j * w:(j + 1) * w]


def _completed(r, done):
    return [(ij, terms) for ij, terms in _SC.items()
            if r in [q for _, q in terms] and all(q in done for _, q in terms)]


def _when_complete(order, product, emit):
    prod = {}
    for r in order:
        prod[r] = product(r)
        for ij, terms in _completed(r, prod):
            terms = [t for t in terms if t[1] == r] + [t for t in terms if t[1] != r]
            emit(*ij, _signed_sum([(s, prod[q]) for s, q in terms]))


def _accumulate(order, product, emit):
    out, done = {}, []
    for r in order:
        val = product(r)
        done.append(r)
        for ij, terms in _SC.items():
            for sign in (s for s, q in terms if q == r):
                out[ij] = (sign, val) if ij not in out else (
                    1, _signed_sum(sorted([out[ij], (sign, val)], key=lambda t: -t[0])))
        for ij, _ in _completed(r, done):
            emit(*ij, out[ij][1])


def _after(never, steps, frac, j, dst):
    src = steps[min(len(steps), math.ceil(frac * len(steps))) - 1]
    r, c = j // 2 * 8 % src.shape[0], j * 128 % src.shape[1]
    src = pltpu.bitcast(src[r:r + 8, c:c + 128], jnp.int32)
    return pltpu.bitcast(jnp.where(never, src, pltpu.bitcast(dst, jnp.int32)), _BF)


def _kernel(x_hbm, wq_hbm, wkt_hbm, wvt_hbm, wo_hbm, wg_hbm, wu_hbm, wd_hbm, gw_hbm, out_hbm,
            wd_v, wo_v, h_v, k_v, kf_v, vt_v, qt_v, g_v, mo_v, zero_s, sems):
    S, D = out_hbm.shape
    F = wg_hbm.shape[1]
    Dh = D // _HEADS
    TR = S // 4
    TC = D // 4
    FC = 2 * TC
    SM = S - 32 * _VPU_GROUPS
    vmem = pltpu.VMEM
    wq_sems, wb_sems = (sems.at[_X_STEPS], sems.at[_X_STEPS + 1]), _X_STEPS + 2
    small_sem, w2_sem, out_sem = (sems.at[_X_STEPS + 4 + i] for i in range(3))

    w2_copies = [pltpu.make_async_copy(src.at[:, :, pl.ds(j * FC, FC)], dst.at[j], w2_sem)
                 for j in range(2) for src, dst in ((wd_hbm, wd_v), (wo_hbm, wo_v))]

    def zeros():
        return [zero_s[u] for u in range(_ZEROS)]

    def spread_keys(b, zero):
        k = pltpu.bitcast(k_v[pl.ds(pl.multiple_of(SM // 2 + 16 * b + zero, 16), 16), :], _BF)
        k = k.astype(_F32)
        for d in range(Dh // 2):
            wide = [jnp.broadcast_to(k[:, c:c + 1], (32, 128)) for c in (d, Dh // 2 + d)]
            for r in range(7):
                kf_v[b][r * Dh // 2 + d] = _factor(_SA[r], lambda i, c: wide[c][16 * i:16 * (i + 1)])

    def projections(x_v, xf_v, wb_v, m_v, kvz_v, ng_v, wkv_v, gw_v, bq_v):
        def x_copy(g):
            return pltpu.make_async_copy(x_hbm.at[:, g], x_v.at[g], sems.at[g])

        def wq_copy(k, j):
            return pltpu.make_async_copy(wq_hbm.at[pl.ds(k * FC, FC), pl.ds(j * FC, FC)],
                                         wb_v.at[1, j, pl.ds(k * FC, FC)], wq_sems[min(1, k + j)])

        def wb_copies(c):
            return [pltpu.make_async_copy(w.at[:, pl.ds(pl.multiple_of(c * FC, FC), FC)],
                                          wb_v.at[c % 2, j], sems.at[wb_sems + c % 2])
                    for j, w in enumerate((wg_hbm, wu_hbm))]

        row_factors = ((3, 5), (7, 1))

        def row_operands(b):
            return jnp.concatenate([b[:128] - b[128:], b[128:]], axis=0).astype(_BF), b.astype(_BF)

        small_copies = [pltpu.make_async_copy(wkt_hbm, wkv_v.at[pl.ds(0, Dh)], small_sem),
                        pltpu.make_async_copy(wvt_hbm, wkv_v.at[pl.ds(Dh, Dh)], small_sem),
                        pltpu.make_async_copy(gw_hbm, gw_v.at[pl.ds(0, D // 128)], small_sem)]
        wq_rest = [wq_copy(1, 0), wq_copy(1, 1), wq_copy(0, 1)]
        for copy in (wq_copy(0, 0), *small_copies, *map(x_copy, range(_X_STEPS)), *wq_rest):
            copy.start()
        for u in range(_ZEROS):
            zero_s[u] = 0
        for m in mo_v:
            m[0] = jnp.zeros((TR, TC), _F32)
        wq_copy(0, 0).wait()
        for r2 in range(7):
            b = _factor(_SB[r2], lambda k, j: wb_v[
                1, 0, pl.ds(k * TC, TC), pl.ds(j * TC, TC)].astype(_F32))
            for i, rhs in enumerate(row_operands(b)):
                bq_v[r2, i] = pltpu.bitcast(rhs, jnp.int32)
        for copy in small_copies:
            copy.wait()
        gw = gw_v[pl.ds(0, D // 128), :].astype(_F32)
        wkv_v[pl.ds(2 * Dh, 128 - 2 * Dh), :] = jnp.concatenate(
            [jnp.broadcast_to(gw[r:r + 1, :], (128 - 2 * Dh, 128)) for r in range(D // 128)],
            axis=1).astype(_BF)

        RG = S // 8 // _X_STEPS

        @pl.loop(0, _X_STEPS)
        def _(g):
            x_copy(g).wait()
            zs, steps, first = zeros(), [], [[] for _ in range(7)]
            for r1 in range(7):
                for lo in range(0, RG, 8):
                    z = zs[(lo // 8 * 7 + r1) % _ZEROS]
                    pair = functools.cache(
                        lambda i, k: x_v[g + z, i, pl.ds(lo, 8), pl.ds(256 * k, 256)].astype(_F32))
                    a1 = _block_factor(
                        _SA[r1], lambda i, k: pair(i, k // 2)[:, k % 2 * 128:k % 2 * 128 + 128], 4)
                    for r2 in range(7):
                        a2 = _block_factor(_SA[r2], a1, 2)
                        a3 = [_factor(terms, a2) for terms in _SA] + [a2(1, 0)]
                        for u in range(4):
                            xf_v[r1][r2, u, pl.ds(pl.multiple_of(g * RG + lo, 8), 8), :] = (
                                jnp.concatenate(a3[2 * u:2 * u + 2], axis=1).astype(_BF))
                        if r1 == 0:
                            first[r2].append(a3)
                        else:
                            steps.append(a3[2])

            def first_product(r2):
                out = []
                for i, (u, w) in enumerate(row_factors):
                    a = [[a3[u], a3[w]] for a3 in first[r2]]
                    for j in range(4):
                        frac = 0.5 + 0.42 * (8 * r2 + 4 * i + j + 1) / 56
                        row = a[j // 2 * 2]
                        row[j % 2] = jnp.where(zs[0] > 0, steps[math.ceil(frac * len(steps)) - 1], row[j % 2])
                    a = jnp.concatenate([jnp.concatenate(row, axis=1) for row in a], axis=0)
                    out.append(_dot(a.astype(_BF), pltpu.bitcast(bq_v[r2, i], _BF)))
                return jnp.concatenate(out, axis=0)

            def first_emit(i2, j2, cur):
                for i in range(2):
                    m_v[2 * i2 + j2][0][0, pl.ds(pl.multiple_of(i * TR // 2 + g * RG, RG), RG), :] = (
                        cur[i * RG:(i + 1) * RG])

            x = x_v[g].reshape(8 * RG, D)
            tiles = [[x[lo:lo + 16, c:c + 128] for c in range(0, D, 128)]
                     for lo in range(0, 8 * RG, 16)]
            n = 8 * len(tiles)
            for j in range(n):
                r, c = j // 4 % len(tiles), j // (n // 2) * 4 + j % 4
                tiles[r][c] = _after(zs[0] > 0, steps, 0.5 * (j + 1) / n, 0, tiles[r][c])
            x = jnp.concatenate([jnp.concatenate(row, axis=1) for row in tiles], axis=0)
            kvz_v[pl.ds(pl.multiple_of(g * 8 * RG, 8 * RG), 8 * RG), :] = _dot_nt(x, wkv_v[...])
            _when_complete(_IN_ORDER, first_product, first_emit)

        def seven_products(n, a, b):
            out = {}
            _accumulate(_INNER_ORDERS[n % 4],
                        lambda r: _dot(a(r), _factor(_SB[r], _quadrants(b)).astype(_BF)),
                        lambda i, j, blk: out.update({(i, j): blk}))
            return jnp.concatenate(
                [jnp.concatenate([out[i, 0], out[i, 1]], axis=1) for i in range(2)], axis=0)

        def eight_products(n, a, b):
            return jnp.concatenate([_dot(jnp.concatenate([a(u), a(w)], axis=1), rhs)
                                    for (u, w), rhs in zip(row_factors, row_operands(b))], axis=0)

        def project(slot, zs, inner, emit, before=lambda r1: None, start=0):
            for r1 in range(start, 7):
                before(r1)

                @functools.cache
                def b1(z):
                    return _block_factor(_SB[r1], lambda k, j: wb_v[
                        slot + zs[z], j // 2, pl.ds(k * TC, TC), pl.ds(j % 2 * TC, TC)].astype(_F32), 2)

                def middle(r2):
                    z = r1 if len(_SB[r1]) > 1 else (7 * r1 + r2) % _ZEROS
                    return inner(7 * r1 + _MIDDLE_ORDERS[r1].index(r2),
                                 lambda r3: xf_v[r1][r2, r3 // 2, :, pl.ds(r3 % 2 * 128, 128)],
                                 _factor(_SB[r2], b1(z)))

                _when_complete(_MIDDLE_ORDERS[r1], middle, functools.partial(emit, r1))

        zs = zeros()

        def before(r1):
            if r1 == 1:
                for copy in wq_rest:
                    copy.wait()
                for copy in wb_copies(0):
                    copy.start()
            if 2 <= r1 < 6:
                t = (r1 + 1) % 4
                kvz = jnp.concatenate([kvz_v[pl.ds((8 * g + b) * RG, RG), :]
                                       for b in (2 * t, 2 * t + 1) for g in range(_X_STEPS)], axis=0)
                k_v[pl.ds(t * TR // 2, TR // 2), :] = pltpu.bitcast(
                    (kvz * (Dh ** -0.5 * math.log2(math.e))).astype(_BF), jnp.int32)
                kvz_t = kvz.T
                vt_v[t] = kvz_t[Dh:2 * Dh].astype(_BF)
                g_v[t] = g = jax.nn.sigmoid(kvz_t[2 * Dh:2 * Dh + 8])
                ng_v[t] = jnp.broadcast_to(1.0 - g[:1], (128, TR)).T
            if r1 == 3:
                spread_keys(0, zs[0])

        def emit_q(r1, i2, j2, cur):
            m = m_v[2 * i2 + j2]
            if r1 not in (4, 6):
                m[r1][0] = cur
            for (i1, j1), terms in _SC.items():
                if terms[0][1] == r1:
                    q = _signed_sum([(s, cur if r == r1 else m[r][zs[r1]]) for s, r in terms])
                    qt_v[2 * i1 + i2, pl.ds((2 * j1 + j2) * TC, TC), :] = q.T.astype(_BF)

        project(1, zs, eight_products, emit_q, before, start=1)

        @pl.loop(0, F // FC)
        def _(c):
            for copy in wb_copies(c):
                copy.wait()

            @pl.when(c + 1 < F // FC)
            def _():
                for copy in wb_copies(c + 1):
                    copy.start()

            zs = zeros()

            def emit_h(r1, i2, j2, cur):
                m = m_v[2 * i2 + j2]

                def get(r):
                    return m[r][zs[r1]]

                if r1 == 2:
                    m[4][0] = cur - get(0)
                    m[2][0] = cur + get(1)
                elif r1 not in (4, 6):
                    m[r1][0] = cur
                elif r1 == 4:
                    gate, up = get(0) + get(1), (cur + get(4)) + get(3)
                    ng = jnp.concatenate([ng_v[2 + i2]] * 2, axis=1)
                    store_h(2 + i2, j2, up * (jnp.maximum(gate, 0.0) * ng))
                else:
                    gate, up = (cur + get(2)) - get(5), get(5) + get(3)
                    ng = jnp.concatenate([ng_v[i2]] * 2, axis=1)
                    store_h(i2, j2, jnp.maximum(gate, 0.0) * (up * ng))

            def store_h(i, j2, h):
                for u in range(2):
                    h_v[i, 4 * c + 2 * j2 + u] = h[:, u * 128:(u + 1) * 128]

            project(c % 2, zs, seven_products, emit_h)

    pl.run_scoped(
        projections,
        vmem((_X_STEPS, 8, S // 8 // _X_STEPS, D), _BF), [vmem((7, 4, S // 8, 256), _BF)] * 7,
        vmem((2, 2, D, FC), _BF), [[vmem((1, TR, TC), _F32)] * 6] * 4, vmem((S, 128), _F32),
        vmem((4, TR, 128), _F32), vmem((128, D), _BF), vmem((64, 128), _BF),
        vmem((7, 2, TC // 2, TC), jnp.int32))

    def attention(ot_v, align_v, qf_v, p_v, l_v, range_v):
        def head_rows(h):
            return pl.ds(pl.multiple_of(h * Dh, Dh), Dh)

        def vpu_probs(q, u, zs):
            half = Dh // 2
            factors = [_factor(terms, _quadrants(q.astype(_F32))) for terms in _SB]
            steps, sums, blocks = [], {}, []
            for b, kf in enumerate(kf_v):
                def product(r):
                    acc = None
                    for d in range(half):
                        col = kf[r * half + d + zs[u]]
                        if b == 0:
                            row = jnp.broadcast_to(factors[r][d:d + 1], (8, TR // 2))
                            qf_v[u][r * half + d] = row
                        else:
                            row = qf_v[u][r * half + d + zs[b]]
                        term = jnp.concatenate([col, col], axis=1) * jnp.concatenate([row, row], axis=0)
                        acc = term if acc is None else acc + term
                        steps.extend([acc] * (4 + (b == 0) + (d == 0)))
                    return acc

                def emit(i, j, s):
                    p = jnp.exp2(s)
                    for part in (p[:8], p[8:]):
                        sums[j] = sums[j] + part if j in sums else part
                    blocks.append((32 * b + 16 * i, 256 * j, p))

                _accumulate(_VPU_ORDERS[b], product, emit)
            return jnp.concatenate([sums[0], sums[1]], axis=1), steps, blocks

        def probs(i, u, zs):
            q = qt_v[u % 4, head_rows(i * (_UNITS // 4) + u // 4), :]
            vpu_sum, steps, blocks = vpu_probs(q, u, zs)
            k = [pltpu.bitcast(k_v[pl.ds(lo, 8), :], _BF) for lo in range(0, SM // 2, 8)]
            for j in range(len(k) - 1):
                frac = (j + 1) / (len(k) - 1)
                k[j] = _after(zs[0] > 0, steps, frac + 0.024 * (1 - frac), j, k[j])
            p = jnp.exp2(_dot(jnp.concatenate(k, axis=0)[:, :Dh], q))
            p_v[u][0, pl.ds(0, SM), :] = p.astype(_BF)
            for r, c, blk in blocks:
                p_v[u][0, pl.ds(SM + r, 16), pl.ds(c, 256)] = blk.astype(_BF)
            l_v[u][0] = jnp.sum(p.reshape(SM // 8, 8, TR), axis=0) + vpu_sum

        def values(h, t, p, l):
            o = _dot(jnp.concatenate([vt_v[w] for w in range(4)], axis=1), p)
            ot_v[t, head_rows(h), :] = o * (g_v[t, :1, :] / l)

        def stored_values(i, u, zs):
            l = jnp.sum(l_v[u][zs[0]], axis=0, keepdims=True)
            values(i * (_UNITS // 4) + u // 4, u % 4, p_v[u][zs[0]], l)
            return l

        def track(sums):
            range_v[0] = functools.reduce(jnp.minimum, sums, range_v[0])
            range_v[1] = functools.reduce(jnp.maximum, sums, range_v[1])

        range_v[...] = jnp.ones_like(range_v)
        align_v[0] = jnp.zeros((8, 128), _F32)

        @pl.when(zero_s[1] == 0)
        def _():
            zs = zeros()
            for b in range(1, len(kf_v)):
                spread_keys(b, zs[0])
            for u in range(_UNITS):
                probs(0, u, zs)

        for copy in w2_copies:
            copy.start()

        @pl.loop(1, 4 * _HEADS // _UNITS)
        def _(i):
            zs, sums = zeros(), []
            for u in range(_UNITS):
                sums.append(stored_values(i - 1, u, zs))
                probs(i, u, zs)
            track(sums)

        zs = zeros()
        track([stored_values(4 * _HEADS // _UNITS - 1, u, zs) for u in range(_UNITS)])

        v_max = jnp.max(jnp.max(jnp.abs(vt_v[...].astype(_F32)), axis=0), keepdims=True)
        v_max = v_max + align_v[zero_s[0], :1, :1]
        safe = ((range_v[0] >= 2.0 ** -40) & (range_v[1] <= 2.0 ** 40)
                & (v_max <= 2.0 ** 80) & ((v_max >= 2.0 ** -50) | (v_max == 0.0)))

        @pl.when(jnp.max(jnp.where(safe, 0.0, 1.0)) > 0.0)
        def _():
            def plain_q(x_v, w_v):
                pltpu.sync_copy(x_hbm, x_v)
                for j in range(4):
                    pltpu.sync_copy(wq_hbm.at[:, pl.ds(j * TC, TC)], w_v.at[j])

                @pl.loop(0, 16)
                def _(n):
                    t, j = n // 4, n % 4
                    q = _dot(x_v[pl.ds(2 * t, 2)].reshape(TR, D), w_v[j])
                    qt_v[t, pl.ds(pl.multiple_of(j * TC, TC), TC), :] = q.T.astype(_BF)

            pl.run_scoped(plain_q, vmem(x_hbm.shape, _BF), vmem((4, D, TC), _BF))

            @pl.loop(0, 4 * _HEADS)
            def _(unit):
                h, t = unit // 4, unit % 4
                s = _dot(pltpu.bitcast(k_v[...], _BF)[:, :Dh], qt_v[t, head_rows(h), :])
                p = jnp.exp2(s - jnp.max(s, axis=0, keepdims=True))
                values(h, t, p.astype(_BF), jnp.sum(p, axis=0, keepdims=True))

    def output(ot_v, out_v):
        pl.run_scoped(functools.partial(attention, ot_v),
                      vmem((3, 8, 128), _F32),
                      [vmem((7 * Dh // 2, 8, TR // 2), _F32)] * _UNITS,
                      [vmem((1, S, TR), _BF)] * _UNITS, [vmem((1, 8, TR), _F32)] * _UNITS,
                      vmem((2, 8, TR), _F32))
        for copy in w2_copies:
            copy.wait()

        def out_copy(i1, j1, i2, j2):
            return pltpu.make_async_copy(
                out_v[2 * i2 + j2].at[2 * i1 + j1],
                out_hbm.at[pl.ds(pl.multiple_of((2 * i1 + i2) * TR, TR), TR),
                           pl.ds(pl.multiple_of((2 * j1 + j2) * TC, TC), TC)], out_sem)

        def factor_spec(terms):
            (_, ia, ja), (sign, ib, jb) = terms[0], terms[-1]
            return (*map(np.int32, (ia, ja, ib, jb)), np.float32(sign if len(terms) == 2 else 0))

        def outer_factor(spec, blk):
            ia, ja, ib, jb, coef = spec
            return functools.cache(
                lambda i2, j2: blk(2 * ia + i2, ja, j2) + coef * blk(2 * ib + i2, jb, j2))

        plan = [None] * 7
        for (i1, j1), terms in _SC.items():
            rest = [r for _, r in terms[1:]]
            plan[terms[0][1]] = (1, i1, j1, *(rest * 3 if len(rest) == 1 else rest))
        for r in reversed(range(7)):
            plan[r] = plan[r] or (0, *plan[r + 1][1:3], 0, 0, 0)
        specs = [(factor_spec(_SA[r]), factor_spec(_SB[r]), tuple(map(np.int32, plan[r])))
                 for r in range(7)]

        def step(spec, keep=None, before=lambda r2: None):
            spec_a, spec_b, (_, i1, j1, ma, mb, mc) = spec
            zs = zeros()
            b1 = outer_factor(spec_b, lambda k, j, j2: jnp.concatenate(
                [w[j, k, :, pl.ds(j2 * TC, TC)].astype(_F32) for w in (wd_v, wo_v)], axis=0))

            @functools.cache
            def a1(z):
                n = F // 4 // 128
                return (outer_factor(spec_a, lambda i, k, k2: jnp.concatenate(
                            [h_v[i + zs[z], (2 * k + k2) * n + u] for u in range(n)], axis=1)),
                        outer_factor(spec_a, lambda i, k, k2: ot_v[
                            i + zs[z], pl.ds(pl.multiple_of((2 * k + k2) * TC, TC), TC), :]))

            def product(r2):
                before(r2)
                h, ot = (_factor(_SA[r2], lambda i, k: a1(r2 if i > k else 7)[w](i, k))
                         for w in range(2))
                a, b = jnp.concatenate([h, ot.T], axis=1), _factor(_SB[r2], b1)
                cuts = list(range(0, b.shape[0], 256)) + [b.shape[0]]
                odd = {2: 4, 6: 2}.get(r2, len(cuts))
                cuts[odd:-1] = [c - 128 for c in cuts[odd:-1]]
                return functools.reduce(jnp.add, (
                    _dot(a[:, lo:hi].astype(_BF), b[lo:hi].astype(_BF))
                    for lo, hi in zip(cuts, cuts[1:])))

            def emit(i2, j2, cur):
                m, n = mo_v[2 * i2 + j2], TR if keep is None else 64
                for lo in range(0, TR, n):
                    rows, part = pl.ds(lo, n), cur[lo:lo + n]
                    val = (part + m[ma, rows]) + (m[mb, rows] - m[mc, rows])
                    out_v[2 * i2 + j2][2 * i1 + j1, rows, :] = val.astype(_BF)
                    if keep is not None:
                        m[keep, rows] = part

            _when_complete(_OUTPUT_ORDER, product, emit)

        @pl.loop(0, 6, init_carry=specs[0])
        def _(r1, spec):
            step(spec, keep=r1)
            final, i1, j1 = spec[2][:3]

            @pl.when(final > 0)
            def _():
                for i2, j2 in _SC:
                    out_copy(i1, j1, i2, j2).start()

            return jax.tree.map(
                lambda *v: functools.reduce(
                    lambda acc, r: jnp.where(r1 + 1 == r, v[r], acc), range(1, 5), v[5]),
                *specs)

        def send_finished_blocks(r2):
            if r2 == 6:
                @pl.loop(0, 1 + zero_s[0])
                def _(_):
                    for i2, j2 in list(_SC)[:3]:
                        out_copy(0, 0, i2, j2).start()

        step(specs[6], before=send_finished_blocks)
        out_copy(0, 0, 0, 0).start()
        for i1, j1 in _SC:
            for i2, j2 in _SC:
                out_copy(i1, j1, i2, j2).wait()

    pl.run_scoped(output, vmem((4, D, TR), _F32), [vmem((4, TR, TC), _BF)] * 4)


@jax.jit
def pallas_gated_mix__grouped_kv_mqa__glu_gated_reglu__prompt_kernel(
    A_x: jax.Array,
    A_wq: jax.Array,
    A_wk: jax.Array,
    A_wv: jax.Array,
    A_wo: jax.Array,
    B_x: jax.Array,
    B_W_gate: jax.Array,
    B_W_up: jax.Array,
    B_W_down: jax.Array,
    gate_w: jax.Array,
):
    del B_x
    B, S, D = A_x.shape
    F = B_W_gate.shape[1]
    Dh, TR, TC = D // _HEADS, S // 4, D // 4
    assert (B, S, D) == (1, 2048, 1024) and F == 3584
    vmem = pltpu.VMEM
    out = pl.pallas_call(
        _kernel,
        out_shape=jax.ShapeDtypeStruct((S, D), _BF),
        in_specs=[pl.BlockSpec(memory_space=pl.ANY)] * 9,
        out_specs=pl.BlockSpec(memory_space=pl.ANY),
        scratch_shapes=[
            vmem((2, 4, F // 4, 2 * TC), _BF),
            vmem((2, 4, TC, 2 * TC), _BF),
            vmem((4, F // 128, TR, 128), _F32),
            vmem((S // 2, 128), jnp.int32),
            [vmem((7 * Dh // 2, 16, 128), _F32)] * _VPU_GROUPS,
            vmem((4, Dh, TR), _BF),
            vmem((4, D, TR), _BF),
            vmem((4, 8, TR), _F32),
            [vmem((7, TR, TC), _F32)] * 4,
            pltpu.SMEM((_ZEROS,), jnp.int32),
            pltpu.SemaphoreType.DMA((_X_STEPS + 7,)),
        ],
        compiler_params=pltpu.CompilerParams(vmem_limit_bytes=127 * 2**20),
        name="gated_mix",
    )(A_x.reshape(8, _X_STEPS, S // 8 // _X_STEPS, D), A_wq, A_wk.T, A_wv.T,
      A_wo.reshape(4, TC, D), B_W_gate, B_W_up, B_W_down.reshape(4, F // 4, D),
      gate_w.reshape(D // 128, 128))
    return out.reshape(B, S, D)
```
